```python
import os as _os
_os.environ.setdefault("JAX_PLATFORMS", "cpu")
import jax
import jax.numpy as jnp

def _softmax(x, axis=-1):
    return jax.nn.softmax(x, axis=axis)
def _gelu(x):
    return jax.nn.gelu(x, approximate=True)
def _silu(x):
    return jax.nn.silu(x)
def _sigmoid(x):
    return jax.nn.sigmoid(x)
def _layernorm(x, axis=-1, eps=1e-5):
    m = jnp.mean(x, axis=axis, keepdims=True)
    v = jnp.var(x, axis=axis, keepdims=True)
    return (x - m) / jnp.sqrt(v + eps)
def _scatter_add(tgt, idx, src, axis=0):
    return tgt.at[idx].add(src)
def _segment_sum(src, seg, n):
    return jax.ops.segment_sum(src, seg, n)
class _Rng:
    def __init__(self, key):
        self._k = key
    def _next(self):
        self._k, sub = jax.random.split(self._k)
        return sub
    def normal(self, shape):
        return jax.random.normal(self._next(), shape, dtype=jnp.bfloat16)
    def randint(self, lo, hi, shape):
        return jax.random.randint(self._next(), shape, lo, hi, dtype=jnp.int32)
    def uniform(self, shape, lo=0.0, hi=1.0):
        return jax.random.uniform(self._next(), shape, jnp.bfloat16, lo, hi)
    def permutation(self, n):
        return jax.random.permutation(self._next(), n)


kernel_name = 'concat_heads__sliding_local_dilated__compressed_kv_cla__prompt'

def setup_inputs():
    _rng = _Rng(jax.random.key(int.from_bytes(__import__("os").urandom(4), "little")))
    _w = (lambda a: (lambda t: t.astype(jnp.bfloat16) if jnp.issubdtype(t.dtype, jnp.floating) else t)(jnp.asarray(a)))
    def _A_setup():
        B, S, D = 1, 2048, 640
        return {
            "x": _w((lambda *s: _rng.normal(s) * 0.2)(B, S, D)),
            "wqkv": _w((lambda *s: _rng.normal(s) * 0.2)(D, 3 * D)),
            "wo": _w((lambda *s: _rng.normal(s) * 0.05)(D, D)),
        }
    _A_in = _A_setup()

    def _B_setup():
        B, H, Sq, Sk, D, M = 1, 32, 2048, 2048, 128, 640
        Dc = 4 * D
        return {
            "x": _w((lambda *s: _rng.normal(s) * 0.8)(B, Sq, M)),
            "c_kv": _w((lambda *s: _rng.normal(s) * 0.8)(B, Sk, Dc)),
            "w_q": _w((lambda *s: _rng.normal(s) * 1.6)(M, H, D) * (M ** -0.5)),
            "w_uk": _w((lambda *s: _rng.normal(s) * 1.6)(Dc, H, D) * (Dc ** -0.5)),
            "w_uv": _w((lambda *s: _rng.normal(s) * 0.8)(Dc, H, D) * (Dc ** -0.5)),
            "w_o": _w((lambda *s: _rng.normal(s) * 0.8)(H, D, M) * ((H * D) ** -0.5)),
        }
    _B_in = _B_setup()

    return {
        "A_x": _A_in["x"],
        "A_wqkv": _A_in["wqkv"],
        "A_wo": _A_in["wo"],
        "B_x": _B_in["x"],
        "B_c_kv": _B_in["c_kv"],
        "B_w_q": _B_in["w_q"],
        "B_w_uk": _B_in["w_uk"],
        "B_w_uv": _B_in["w_uv"],
        "B_w_o": _B_in["w_o"],
    }

def reference(A_x, A_wqkv, A_wo, B_x, B_c_kv, B_w_q, B_w_uk, B_w_uv, B_w_o):
    def _A_ref(x, wqkv, wo):
        B, S, D = x.shape
        H = 32; Dh = D // H
        W, dil = 8, 2
        qkv = (lambda x, *d: x.transpose(*d))((x @ wqkv).reshape(B, S, 3, H, Dh), 2, 0, 3, 1, 4)
        q, k, v = qkv[0], qkv[1], qkv[2]
        scale = Dh ** -0.5
        pos = jnp.arange(S)
        off = jnp.arange(W) * dil
        idx = pos[:, None] - off[None, :]
        mask = idx >= 0
        idx_c = jnp.where(mask, idx, 0).reshape(-1)
        kg = k[:, :, idx_c, :].reshape(B, H, S, W, Dh)
        vg = v[:, :, idx_c, :].reshape(B, H, S, W, Dh)
        logits = jnp.einsum("bhsd,bhswd->bhsw", q, kg) * scale
        logits = jnp.where(mask[None, None, :, :], logits, -1e9)
        attn = _softmax(logits, axis=-1)
        o = jnp.einsum("bhsw,bhswd->bhsd", attn, vg)
        return (lambda x, *d: x.transpose(*d))(o, 0, 2, 1, 3).reshape(B, S, D) @ wo

    def _B_ref(x, c_kv, w_q, w_uk, w_uv, w_o):
        B, Sq, M = x.shape[0], x.shape[1], x.shape[2]
        Sk = c_kv.shape[1]
        H, D = w_q.shape[1], w_q.shape[2]
        q = jnp.einsum("bqm,mhd->bhqd", x, w_q)
        k = jnp.einsum("bkc,chd->bhkd", c_kv, w_uk)
        v = jnp.einsum("bkc,chd->bhkd", c_kv, w_uv)
        scores = jnp.einsum("bhqd,bhkd->bhqk", q, k) * (D ** -0.5)
        off = Sk - Sq
        qi = jnp.arange(Sq)[:, None]
        kj = jnp.arange(Sk)[None, :]
        cmask = kj <= (qi + off)
        scores = jnp.where(cmask[None, None], scores, -1e9)
        p = _softmax(scores, axis=-1)
        ctx = jnp.einsum("bhqk,bhkd->bhqd", p, v)
        return jnp.einsum("bhqd,hdm->bqm", ctx, w_o)

    a = _A_ref(A_x, A_wqkv, A_wo)
    b = _B_ref(B_x, B_c_kv, B_w_q, B_w_uk, B_w_uv, B_w_o)
    return jnp.concatenate([a, b], axis=-1)
```

```python
import functools
import math

import jax
import jax.numpy as jnp
from jax import lax
import jax.experimental.pallas as pl
import jax.experimental.pallas.tpu as pltpu

S = 2048
DM = 640
H = 32
HD = 128
DC = 512
AH = 32
ADH = 20
AW = 8
BQ = 512
T = 128
AC = 256
UPAD = 2
RG = 32
LOG2E = math.log2(math.e)
F32 = jnp.float32
BF16 = jnp.bfloat16
NT = (((1,), (1,)), ((), ()))


def _dot(a, b):
    return jnp.dot(a, b, preferred_element_type=F32)


def _pair(u_ref, j):
    rows = u_ref.shape[1] * (H // 4)
    start = (j // (H // 4)) * rows + j % (H // 4)
    u = u_ref.reshape(2 * rows, HD)[pl.ds(start, u_ref.shape[1] - UPAD, stride=H // 4), :]
    lo = pltpu.bitcast(u << 16, F32).astype(BF16)
    hi = pltpu.bitcast(u & jnp.uint32(0xFFFF0000), F32).astype(BF16)
    return jnp.concatenate([lo, hi], axis=1)


def _part_a(ax_ref, wqkv_ref, wo_ref, o_ref, kv_ref, att_ref, tmp_ref, wt_ref, wait_wqkv, wait_w, wait_x, before_last):
    def permute_rows(w, dst):
        for t in range(5):
            tmp_ref[t, 0:DM, :] = w[:, t * 128:(t + 1) * 128].astype(F32)
        for d in range(ADH):
            blk = [tmp_ref[t, pl.ds(d, AH, stride=ADH), :] for t in range(5)]
            dst[d * AH:(d + 1) * AH, :] = jnp.concatenate(blk, axis=1).astype(BF16)

    def permute(i, carry):
        wait_wqkv(i)
        permute_rows(wqkv_ref[i].T, wt_ref.at[i])
        return carry

    lax.fori_loop(0, 3, permute, 0)
    wait_w()
    kv_ref[5:15, 0:16, :] = jnp.zeros((10, 16, 128), F32)

    def project(r0, d=None):
        x = ax_ref[pl.ds(r0, AC), :]
        for g in range(3):
            y = lax.dot_general(_after(x, d if g >= 1 else None), wt_ref[g], NT, preferred_element_type=F32)
            if g == 0:
                y = y * (ADH ** -0.5 * LOG2E)
            for t in range(5):
                kv_ref[5 * g + t, pl.ds(16 + r0, AC), :] = y[:, t * 128:(t + 1) * 128]

    def attend1(r0, par):
        ld = lambda t, off: kv_ref[t, pl.ds(16 + r0 - off, RG), :]
        row = lax.broadcasted_iota(jnp.int32, (RG, 128), 0) + r0
        ls = []
        for w in range(AW):
            a = None
            for t in range(5):
                p = ld(t, 0) * ld(5 + t, 2 * w)
                a = p if a is None else a + p
            a = a + pltpu.roll(a, 64, 1)
            a = a + pltpu.roll(a, 32, 1)
            if w > 0:
                a = jnp.where(row >= 2 * w, a, -1e9)
            ls.append(a)
        m = functools.reduce(jnp.maximum, ls)
        es = [jnp.exp2(a - m) for a in ls]
        inv = _recip(functools.reduce(lambda a, b: a + b, es))
        for t in range(5):
            o = None
            for w in range(AW):
                p = es[w] * ld(10 + t, 2 * w)
                o = p if o is None else o + p
            att_ref[t, pl.ds(par, RG), :] = o * inv

    def attend(r0):
        for g in range(0, AC, RG):
            attend1(r0 + g, g)
        return jnp.concatenate([att_ref[t] for t in range(5)], axis=1).astype(BF16)

    def body(ci, carry):
        r0 = pl.multiple_of(ci * AC, AC)
        att = attend(r0)
        project(r0 + AC, att_ref[0, AC // 2:AC // 2 + 16, :])
        o_ref[pl.ds(r0, AC), :] = _dot(att, wo_ref[...]).astype(BF16)
        return carry

    project(0)
    permute_rows(wo_ref[...], wo_ref)
    wait_x()
    lax.fori_loop(0, S // AC - 1, body, 0)
    before_last()
    att = attend(S - AC)
    for h in range(2):
        o_ref[S - AC + h * AC // 2:S - AC + (h + 1) * AC // 2, :] = _dot(
            att[h * AC // 2:(h + 1) * AC // 2], wo_ref[...]).astype(BF16)


def _recip(x):
    r = pl.reciprocal(x, approx=True)
    return r + r * (1.0 - x * r)


def _tail(full, part, op, r):
    if r == 0:
        return op(full, part)
    return jnp.concatenate([full[:r], op(full[r:], part)], axis=0)


def _fold(a, op):
    return functools.reduce(op, [a[:, t * 128:(t + 1) * 128] for t in range(a.shape[1] // 128)])


def _after(a, b):
    if b is None:
        return a
    true = (pltpu.bitcast(b[:16, :128], jnp.int32) | 1) != 0
    a0 = jnp.where(true, a[:16, :128].astype(F32), 0.0).astype(a.dtype)
    if a.shape[1] > 128:
        a0 = jnp.concatenate([a0, a[:16, 128:]], axis=1)
    return jnp.concatenate([a0, a[16:]], axis=0)


def _attn_block(q_s, k_s, v_s, r0, hs, filler, late, p_ref):
    row = lax.broadcasted_iota(jnp.int32, (T, T), 0)
    col = lax.broadcasted_iota(jnp.int32, (T, T), 1)
    sd = []
    for c in range(BQ // T):
        a = r0 + c * T
        s = lax.dot_general(q_s[a:r0 + BQ, hs], k_s[a:a + T, hs], NT, preferred_element_type=F32)
        top = jnp.where(col <= row, s[:T], -1e9)
        sd.append(top if c == BQ // T - 1 else jnp.concatenate([top, s[T:]], axis=0))
    mt = _fold(sd[0], jnp.maximum)
    for c in range(1, BQ // T):
        mt = _tail(mt, _fold(sd[c], jnp.maximum), jnp.maximum, c * T)
    if r0 > 0:
        sm = lax.dot_general(_after(q_s[r0:r0 + BQ, hs], s), k_s[0:r0, hs], NT, preferred_element_type=F32)
        mt = jnp.maximum(mt, _fold(sm, jnp.maximum))
    m = jnp.max(mt, axis=1, keepdims=True)
    f = filler(mt if r0 >= 1024 else sm if r0 > 0 else sd[-1])
    late(jnp.broadcast_to(m, (BQ, 128)))
    lt = o = None
    for c in range(BQ // T):
        a = r0 + c * T
        p = jnp.exp2(sd[c] - m[c * T:])
        oc = _dot(_after(p.astype(BF16), None), v_s[a:a + T, hs])
        lc = _fold(p, jnp.add)
        lt = lc if lt is None else _tail(lt, lc, jnp.add, c * T)
        o = oc if o is None else _tail(o, oc, jnp.add, c * T)
    if r0 > 0:
        p = jnp.exp2(sm - m)
        lt = lt + _fold(p, jnp.add)
        p = p.astype(BF16)
        if (r0, hs.start) == (S - BQ, HD):
            p_ref[:, 0:r0] = p
            p = p_ref[:, 0:r0]
        oc = _dot(p, v_s[0:r0, hs])
        o = o + oc
    l = jnp.sum(lt, axis=1, keepdims=True)
    return (o * _recip(l)).astype(BF16), oc


def _kernel(ax_h, wqkv_h, awo_h, x_h, c_h, wq_h, wk_h, wv_h, wo_h, o_h,
            ax_ref, wqkv_ref, awo_ref, x_ref, c_ref, uq, uk, uv, wo_ref, oa_s, ob_s,
            q_s, k_s, v_s, ctx_s, acc_ref, kv_ref, att_ref, tmp_ref, wt_ref, wq_s, wk_s, wv_s, p_s, sems):
    cp = lambda src, dst, i: pltpu.make_async_copy(src, dst, sems.at[i])
    c_wqkv = lambda i: cp(wqkv_h.at[:, pl.ds(pl.multiple_of(i * DM, 128), DM)],
                          wqkv_ref.at[i], i)
    c_awo = cp(awo_h, awo_ref, 3)
    c_ax0, c_ax = cp(ax_h.at[0:AC], ax_ref.at[0:AC], 8), cp(ax_h.at[AC:S], ax_ref.at[AC:S], 4)
    c_x, c_c = cp(x_h, x_ref, 5), cp(c_h, c_ref, 6)
    c_oa = cp(oa_s, o_h.at[:, 0:DM], 7)
    c_rows = lambda i: slice((0, 512, 1024, 1536, 1792)[i], (512, 1024, 1536, 1792, 2048)[i])
    c_ob = lambda i: cp(ob_s.at[c_rows(i)], o_h.at[c_rows(i), DM:2 * DM], 18 + i)

    def c_w(half):
        ps, hs = pl.ds(8 * half, 8), pl.ds(16 * half, 16)
        return [cp(h.bitcast(jnp.uint32).at[:, ps, :], u.at[half, 0:h.shape[0]], 10 + 4 * half + i)
                for i, (h, u) in enumerate(((wq_h, uq), (wk_h, uk), (wv_h, uv)))] + [
                cp(wo_h.at[hs], wo_ref.at[hs], 13 + 4 * half)]

    def extract(jn, slot):
        wq_s[slot] = _pair(uq, jn); wk_s[slot] = _pair(uk, jn); wv_s[slot] = _pair(uv, jn)

    def wo(j):
        return wo_ref[pl.ds(2 * j, 2)].reshape(2 * HD, DM)

    def rows(i):
        a, b = i if isinstance(i, tuple) else (i, i + 1)
        return slice(a * BQ, b * BQ)

    c_wqkv(0).start()
    c_wqkv(1).start()
    acc_ref[...] = jnp.zeros_like(acc_ref)
    ctx_s[S - BQ:] = jnp.zeros((BQ, 2 * HD), BF16)

    def before_last():
        for c in [c_x, c_c] + c_w(0):
            c.wait()
        for c in c_w(1):
            c.start()

    def wait_wqkv(i):
        c_wqkv(i).wait()

        @pl.when(i == 0)
        def _():
            for c in [c_wqkv(2), c_ax0, c_awo]:
                c.start()

    def wait_x():
        c_ax.wait()
        for c in [c_x, c_c] + c_w(0):
            c.start()

    _part_a(ax_ref, wqkv_ref, awo_ref, oa_s, kv_ref, att_ref, tmp_ref, wt_ref, wait_wqkv,
            lambda: (c_ax.start(), c_ax0.wait(), c_awo.wait()), wait_x,
            before_last)
    extract(0, 0)
    c_oa.start()

    def step(j, carry):
        @pl.when(j == H // 4 - 1)
        def _():
            for c in c_w(1):
                c.wait()

        def pq(i, d):
            r = _dot(_after(x_ref[rows(i)], d), wq_s[j % 2])
            q_s[rows(i)] = (r * (HD ** -0.5 * LOG2E)).astype(BF16)
            return r

        def pk(i, d):
            r = _dot(_after(c_ref[rows(i)], d), wk_s[j % 2])
            k_s[rows(i)] = r.astype(BF16)
            return r

        def pv(i, d):
            r = _dot(_after(c_ref[rows(i)], d), wv_s[j % 2])
            v_s[rows(i)] = r.astype(BF16)
            return r

        def po(i, d):
            r = _dot(_after(ctx_s[rows(i)], d), wo(j))
            acc_ref[rows(i)] += r
            return r

        def attn(prev, i, hh, *fill, late=lambda d: None):
            def filler(d):
                for fn, arg in fill:
                    d = fn(arg, d)
                return d
            hs = slice(hh * HD, (hh + 1) * HD)
            ctx_s[rows(i), hs], d = _attn_block(q_s, k_s, v_s, i * BQ, hs, filler, late, p_s.at[hh])
            return d

        extract(jnp.minimum(j + 1, H // 2 - 1), (j + 1) % 2)
        acc_ref[rows(3)] += _dot(ctx_s[rows(3)], wo(jnp.maximum(j - 1, 0)))
        d = pv(0, pk(0, pq(0, None)))
        d = attn(d, 0, 0, (pq, (1, 3))); d = attn(d, 0, 1, (pk, 1), (pv, 1))
        d = attn(d, 1, 0, (pk, (2, 4))); d = attn(d, 1, 1, (pv, 2))
        d = attn(d, 2, 0, (pv, 3)); d = attn(d, 2, 1, (pq, 3))
        d = attn(d, 3, 0, (po, 0)); d = attn(d, 3, 1, (po, 1), late=lambda d: po(2, d[256:]))

        return carry

    lax.fori_loop(0, H // 2, step, 0)
    c_oa.wait()
    for i in range(3):
        ob_s[rows(i)] = acc_ref[rows(i)].astype(BF16)
        c_ob(i).start()
    for i in (3, 4):
        r = c_rows(i)
        ob_s[r] = (acc_ref[r] + _dot(ctx_s[r], wo(H // 2 - 1))).astype(BF16)
        c_ob(i).start()
    for i in range(5):
        c_ob(i).wait()


@jax.jit
def pallas_concat_heads__sliding_local_dilated__compressed_kv_cla__prompt_kernel(
        A_x, A_wqkv, A_wo, B_x, B_c_kv, B_w_q, B_w_uk, B_w_uv, B_w_o):
    hbm = pl.BlockSpec(memory_space=pl.ANY)
    out = pl.pallas_call(
        _kernel,
        in_specs=[hbm] * 9,
        out_specs=hbm,
        out_shape=jax.ShapeDtypeStruct((S, 2 * DM), BF16),
        scratch_shapes=[
            pltpu.VMEM((S, DM), BF16), pltpu.VMEM((3, DM, DM), BF16), pltpu.VMEM((DM, DM), BF16),
            pltpu.VMEM((S, DM), BF16), pltpu.VMEM((S, DC), BF16),
            pltpu.VMEM((2, DM + UPAD, H // 4, HD), jnp.uint32), pltpu.VMEM((2, DC + UPAD, H // 4, HD), jnp.uint32),
            pltpu.VMEM((2, DC + UPAD, H // 4, HD), jnp.uint32), pltpu.VMEM((H, HD, DM), BF16),
            pltpu.VMEM((S, DM), BF16), pltpu.VMEM((S, DM), BF16),
            pltpu.VMEM((S, 2 * HD), BF16), pltpu.VMEM((S, 2 * HD), BF16), pltpu.VMEM((S, 2 * HD), BF16),
            pltpu.VMEM((S, 2 * HD), BF16), pltpu.VMEM((S, DM), F32), pltpu.VMEM((15, S + 16, 128), F32), pltpu.VMEM((5, AC, 128), F32),
            pltpu.VMEM((5, DM + 32, 128), F32), pltpu.VMEM((3, DM, DM), BF16),
            pltpu.VMEM((2, DM, 2 * HD), BF16), pltpu.VMEM((2, DC, 2 * HD), BF16), pltpu.VMEM((2, DC, 2 * HD), BF16),
            pltpu.VMEM((2, BQ, S - BQ), BF16), pltpu.SemaphoreType.DMA((23,)),
        ],
        compiler_params=pltpu.CompilerParams(
            vmem_limit_bytes=110 * 1024 * 1024),
    )(A_x[0], A_wqkv, A_wo, B_x[0], B_c_kv[0], B_w_q, B_w_uk, B_w_uv, B_w_o)
    return out[None]
```
